```python
import jax
import jax.numpy as jnp

def _softmax(x, axis=-1):
    return jax.nn.softmax(x, axis=axis)
def _gelu(x):
    return jax.nn.gelu(x, approximate=True)
def _silu(x):
    return jax.nn.silu(x)
def _sigmoid(x):
    return jax.nn.sigmoid(x)
def _layernorm(x, axis=-1, eps=1e-5):
    m = jnp.mean(x, axis=axis, keepdims=True)
    v = jnp.var(x, axis=axis, keepdims=True)
    return (x - m) / jnp.sqrt(v + eps)
def _scatter_add(tgt, idx, src, axis=0):
    return tgt.at[idx].add(src)
def _segment_sum(src, seg, n):
    return jax.ops.segment_sum(src, seg, n)
class _Rng:
    def __init__(self, key):
        self._k = key
    def _next(self):
        self._k, sub = jax.random.split(self._k)
        return sub
    def normal(self, shape):
        return jax.random.normal(self._next(), shape, dtype=jnp.bfloat16)
    def randint(self, lo, hi, shape):
        return jax.random.randint(self._next(), shape, lo, hi, dtype=jnp.int32)
    def uniform(self, shape, lo=0.0, hi=1.0):
        return jax.random.uniform(self._next(), shape, jnp.bfloat16, lo, hi)
    def permutation(self, n):
        return jax.random.permutation(self._next(), n)


kernel_name = 'parallel_sum__sliding_block_cached__moe_arch_mod__decode'

def setup_inputs():
    _rng = _Rng(jax.random.key(int.from_bytes(__import__("os").urandom(4), "little")))
    _w = (lambda a: (lambda t: t.astype(jnp.bfloat16) if jnp.issubdtype(t.dtype, jnp.floating) else t)(jnp.asarray(a)))
    def _A_setup():
        B, Sq, D = 1, 1, 512
        Hq, Hkv, Sk, Dh = 32, 8, 65536, 128
        assert Hq % Hkv == 0, (Hq, Hkv)
        return {
            "x": _w((lambda *s: _rng.normal(s) * 0.05)(B, Sq, D)),
            "k_cache": _w((lambda *s: _rng.normal(s) * 0.05)(B, Hkv, Sk, Dh)),
            "v_cache": _w((lambda *s: _rng.normal(s) * 0.05)(B, Hkv, Sk, Dh)),
            "wq": _w((lambda *s: _rng.normal(s) * 0.05)(D, Hq * Dh) * (D ** -0.5)),
            "wo": _w((lambda *s: _rng.normal(s) * 0.05)(Hq * Dh, D) * ((Hq * Dh) ** -0.5)),
        }
    _A_in = _A_setup()

    def _B_setup():
        B, S, D, F, C = 1, 1, 512, 1792, 1
        return {
            "x": _w((lambda *s: _rng.normal(s) * 0.05)(B, S, D)),
            "w_r": _w((lambda *s: _rng.normal(s) * 0.05)(D)),
            "w_gate": _w((lambda *s: _rng.normal(s) * 0.05)(D, F)),
            "w_up": _w((lambda *s: _rng.normal(s) * 0.05)(D, F)),
            "w_down": _w((lambda *s: _rng.normal(s) * 0.05)(F, D)),
        }
    _B_in = _B_setup()

    return {
        "A_x": _A_in["x"],
        "A_k_cache": _A_in["k_cache"],
        "A_v_cache": _A_in["v_cache"],
        "A_wq": _A_in["wq"],
        "A_wo": _A_in["wo"],
        "B_x": _B_in["x"],
        "B_w_r": _B_in["w_r"],
        "B_w_gate": _B_in["w_gate"],
        "B_w_up": _B_in["w_up"],
        "B_w_down": _B_in["w_down"],
    }

def reference(A_x, A_k_cache, A_v_cache, A_wq, A_wo, B_x, B_w_r, B_w_gate, B_w_up, B_w_down):
    def _A_ref(x, k_cache, v_cache, wq, wo):
        B, Sq, D = x.shape
        Hq, Dh = 32, 128
        Hkv, Sk = k_cache.shape[1], k_cache.shape[2]
        W = min(4096, max(256, Sk // 4))
        rep = Hq // Hkv
        q = (lambda x, *d: x.transpose(*d))((x @ wq).reshape(B, Sq, Hq, Dh), 0, 2, 1, 3)
        k = jnp.repeat(k_cache[:, :, Sk - W:, :], rep, axis=1)
        v = jnp.repeat(v_cache[:, :, Sk - W:, :], rep, axis=1)
        scores = jnp.einsum("bhqd,bhkd->bhqk", q, k) * (Dh ** -0.5)
        p = _softmax(scores, axis=-1)
        o = jnp.einsum("bhqk,bhkd->bhqd", p, v)
        return (lambda x, *d: x.transpose(*d))(o, 0, 2, 1, 3).reshape(B, Sq, Hq * Dh) @ wo

    def _B_ref(x, w_r, w_gate, w_up, w_down):
        B, S, D = x.shape
        C = 1
        r = x @ w_r
        idx = jnp.argsort(-r, axis=-1)[:, :C]
        idx_e = jnp.repeat(idx.reshape(B, C, 1), D, axis=2)
        x_sel = jnp.take_along_axis(x, idx_e, axis=1)
        g = _silu(x_sel @ w_gate)
        u = x_sel @ w_up
        y = (g * u) @ w_down
        r_sel = _sigmoid(jnp.take_along_axis(r, idx, axis=1))
        y = y * r_sel.reshape(B, C, 1)
        b_off = (jnp.arange(B) * S).reshape(B, 1)
        flat_idx = (idx + b_off).reshape(B * C)
        zero = (x * 0.0).reshape(B * S, D)
        upd = _scatter_add(zero, flat_idx, y.reshape(B * C, D), axis=0)
        return x + upd.reshape(B, S, D)

    x = A_x
    xn = _layernorm(x, axis=-1)
    return x + _A_ref(xn, A_k_cache, A_v_cache, A_wq, A_wo) + _B_ref(xn, B_w_r, B_w_gate, B_w_up, B_w_down)
```

```python
import jax
import jax.numpy as jnp
from jax import lax
import jax.experimental.pallas as pl
import jax.experimental.pallas.tpu as pltpu

_HQ, _DH = 32, 128
_BF16, _F32 = jnp.bfloat16, jnp.float32
_WINDOW = 192
_STREAMS = 8
_O_FAR = 3


def _dot(a, b):
    return lax.dot_general(a, b, (((1,), (0,)), ((), ())), preferred_element_type=_F32)


def _dot_nt(a, b):
    return lax.dot_general(a, b, (((1,), (1,)), ((), ())), preferred_element_type=_F32)


def _rows(r0, nr, c0=None, nc=None):
    cols = slice(None) if c0 is None else pl.ds(c0, nc)
    return (pl.ds(r0, nr), cols)


class _CopyStream:
    def __init__(self, src, dst, sems, window):
        self.src, self.dst, self.sems, self.window = src, dst, sems, window
        self.copies = []
        self.groups = {}
        self.sem_of = {}
        self.started = 0
        self.done = 0
        self.waited = set()

    def add(self, name, src_idx, dst_idx, group):
        if group not in self.groups:
            self.groups[group] = []
            self.sem_of[group] = len(self.sem_of)
        self.groups[group].append(len(self.copies))
        self.copies.append((name, src_idx, dst_idx, group))

    def add_round_robin(self, streams, group_of):
        for r in range(max(len(s) for s in streams)):
            for j, s in enumerate(streams):
                if r < len(s):
                    self.add(*s[r], group_of(r, j))

    def _copy(self, i):
        name, src_idx, dst_idx, group = self.copies[i]
        return pltpu.make_async_copy(
            self.src[name].at[src_idx], self.dst[name].at[dst_idx], self.sems.at[self.sem_of[group]])

    def start_next(self):
        i = self.started
        self._copy(i).start(priority=i % 2)
        self.started += 1

    def fill(self):
        while self.started < len(self.copies) and self.started - self.done < self.window:
            self.start_next()

    def wait(self, group):
        if group in self.waited:
            return
        ids = self.groups[group]
        while self.started <= ids[-1]:
            self.start_next()
        for i in ids:
            self._copy(i).wait()
        self.waited.add(group)
        self.done += len(ids)
        self.fill()


def _plan(d, f, hkv, sk, w):
    ns = _STREAMS
    hq_dh = _HQ * _DH

    def same(name, idx):
        return (name, idx, idx)

    per = d // ns
    q_phase = [[same("wq", _rows(per * j + 8 * t, 8, (hq_dh // 2) * c, hq_dh // 2))
                for t in range(per // 8) for c in range(2)] for j in range(ns)]
    kv_phases = []
    for g in range(0, hkv, ns // 2):
        kv_phases.append([
            [(name, (0, h, pl.ds(sk - w + 128 * r, 128), slice(None)), (h, pl.ds(128 * r, 128), slice(None)))
             for r in range(w // 128)]
            for h in range(g, g + ns // 2) for name in ("k", "v")])
    per = d // (ns // 2)
    gu_phase = [[same(name, _rows(per * j + 8 * t, 8)) for t in range(per // 8)]
                for j in range(ns // 2) for name in ("wg", "wu")]
    per = f // ns
    d_phase = [[same("wd", _rows(per * j + 32 * r, 32)) for r in range(per // 32)] for j in range(ns)]
    o_phase = [[same("wo", _rows(_DH * _O_FAR * j + 32 * r, 32)) for r in range(4 * _O_FAR)]
               for j in range(ns)]
    return q_phase, kv_phases, gu_phase, d_phase, o_phase


def _kernel(x_hbm, k_hbm, v_hbm, wq_hbm, wo_hbm, wr_hbm, wg_hbm, wu_hbm, wd_hbm, o_ref,
            x_buf, wr_buf, wq_buf, k_buf, v_buf, wo_buf, wg_buf, wu_buf, wd_buf, sems, small_sems):
    d = x_hbm.shape[-1]
    f = wg_hbm.shape[-1]
    hkv, sk = k_hbm.shape[1], k_hbm.shape[2]
    w = k_buf.shape[1]
    rep = _HQ // hkv
    ns = _STREAMS

    stream = _CopyStream(
        dict(k=k_hbm, v=v_hbm, wq=wq_hbm, wo=wo_hbm, wg=wg_hbm, wu=wu_hbm, wd=wd_hbm),
        dict(k=k_buf, v=v_buf, wq=wq_buf, wo=wo_buf, wg=wg_buf, wu=wu_buf, wd=wd_buf),
        sems, _WINDOW)
    q_phase, kv_phases, gu_phase, d_phase, o_phase = _plan(d, f, hkv, sk, w)
    rounds = []

    def by_round(tag):
        def group_of(r, _):
            if (tag, r) not in rounds:
                rounds.append((tag, r))
            return (tag, r)
        return group_of

    stream.add_round_robin(q_phase, by_round("q"))
    for g, phase in enumerate(kv_phases):
        stream.add_round_robin(phase, by_round(("kv", g)))
    stream.add_round_robin(gu_phase, by_round("gu"))
    stream.add_round_robin(d_phase, by_round("d"))
    assert len(stream.copies) % 2 == 0
    stream.add_round_robin(o_phase, lambda r, j: ("o", r // 4, j % 2))
    tail0 = ns * _O_FAR
    n_pairs = (_HQ - tail0) // 2
    for pr in range(n_pairs):
        for c in range(4):
            for par in range(2):
                idx = _rows(_DH * (tail0 + 2 * pr + par) + 32 * c, 32)
                stream.add("wo", idx, idx, ("t", pr, par))

    def far(u, par):
        return [(("o", u, par), [_O_FAR * j + u for j in range(par, ns, 2)])]

    def tail(pr, par):
        return [(("t", pr, par), [tail0 + 2 * pr + par])]

    units = []
    for u in range(_O_FAR - 1):
        units += [far(u, 0), far(u, 1)]
    units += [far(_O_FAR - 1, 0), sum((tail(pr, 0) for pr in range(n_pairs)), []), far(_O_FAR - 1, 1)]
    units += [tail(pr, 1) for pr in range(n_pairs)]
    units = [([g for g, _ in u], [h for _, hs in u for h in hs]) for u in units]

    def need(tag):
        last = [g for g in rounds if g[0] == tag][-1]
        for g in rounds:
            stream.wait(g)
            if g == last:
                break

    x_copy = pltpu.make_async_copy(x_hbm, x_buf, small_sems.at[0])
    wr_copy = pltpu.make_async_copy(wr_hbm, wr_buf, small_sems.at[1])
    for _ in range(ns):
        stream.start_next()
    x_copy.start()
    wr_copy.start()
    stream.fill()
    x_copy.wait()
    wr_copy.wait()

    x = x_buf[0].astype(_F32)
    xc = x - jnp.mean(x, axis=-1, keepdims=True)
    var = jnp.mean(xc * xc, axis=-1, keepdims=True)
    xn = (xc / jnp.sqrt(var + 1e-5)).astype(_BF16).astype(_F32)
    w_r = wr_buf[...].astype(_F32).reshape(1, d)
    gate = jax.nn.sigmoid(jnp.sum(xn * w_r, axis=-1, keepdims=True))
    xn8 = jnp.broadcast_to(xn, (8, d)).astype(_BF16)

    need("q")
    q = _dot(xn8, wq_buf[...])
    head_row = lax.broadcasted_iota(jnp.int32, (8, _DH), 0) % rep
    scale = _DH ** -0.5
    heads_out = []
    for g in range(len(kv_phases)):
        need(("kv", g))
        for h in range(g * (ns // 2), (g + 1) * (ns // 2)):
            q_g = q[:, rep * h * _DH:(rep * h + 1) * _DH]
            for r in range(1, rep):
                q_g = jnp.where(head_row == r, q[:, (rep * h + r) * _DH:(rep * h + r + 1) * _DH], q_g)
            s = _dot_nt(q_g.astype(_BF16), k_buf[h]) * scale
            p = jnp.exp(s - jnp.max(s, axis=-1, keepdims=True))
            denom = jnp.sum(p, axis=-1, keepdims=True)
            o = _dot(p.astype(_BF16), v_buf[h]) / denom
            heads_out.append(o.astype(_BF16).astype(_F32))

    need("gu")
    g_act = jax.nn.silu(_dot(xn8, wg_buf[...]))
    act = (g_act * _dot(xn8, wu_buf[...])).astype(_BF16)
    need("d")
    y = _dot(act, wd_buf[...])

    def head(h):
        return jnp.broadcast_to(heads_out[h // rep][h % rep:h % rep + 1, :], (8, _DH))

    lhs = [jnp.concatenate([head(h) for h in hs], axis=1).astype(_BF16) for _, hs in units]
    acc = jnp.broadcast_to(x + xn, (8, d)) + y * gate
    for (groups, hs), a in zip(units, lhs):
        for g in groups:
            stream.wait(g)
        acc = acc + _dot(a, jnp.concatenate([wo_buf[pl.ds(_DH * h, _DH), :] for h in hs], axis=0))
    assert stream.done == len(stream.copies)
    o_ref[0] = acc[0:1, :].astype(o_ref.dtype)


@jax.jit
def pallas_parallel_sum__sliding_block_cached__moe_arch_mod__decode_kernel(
    A_x: jax.Array,
    A_k_cache: jax.Array,
    A_v_cache: jax.Array,
    A_wq: jax.Array,
    A_wo: jax.Array,
    B_x: jax.Array,
    B_w_r: jax.Array,
    B_w_gate: jax.Array,
    B_w_up: jax.Array,
    B_w_down: jax.Array,
):
    del B_x
    b, sq, d = A_x.shape
    _, hkv, sk, dh = A_k_cache.shape
    f = B_w_gate.shape[-1]
    w = min(4096, max(256, sk // 4))
    assert (b, sq, dh, hkv) == (1, 1, _DH, _STREAMS) and A_wq.shape == (d, _HQ * _DH)
    hbm = pl.BlockSpec(memory_space=pl.ANY)
    return pl.pallas_call(
        _kernel,
        out_shape=jax.ShapeDtypeStruct((b, sq, d), A_x.dtype),
        in_specs=[hbm] * 9,
        out_specs=pl.BlockSpec(memory_space=pltpu.VMEM),
        scratch_shapes=[
            pltpu.VMEM((b, sq, d), _BF16),
            pltpu.VMEM((d,), _BF16),
            pltpu.VMEM((d, _HQ * _DH), _BF16),
            pltpu.VMEM((hkv, w, dh), _BF16),
            pltpu.VMEM((hkv, w, dh), _BF16),
            pltpu.VMEM((_HQ * _DH, d), _BF16),
            pltpu.VMEM((d, f), _BF16),
            pltpu.VMEM((d, f), _BF16),
            pltpu.VMEM((f, d), _BF16),
            pltpu.SemaphoreType.DMA((144,)),
            pltpu.SemaphoreType.DMA((2,)),
        ],
        compiler_params=pltpu.CompilerParams(
            vmem_limit_bytes=48 * 1024 * 1024,
            disable_semaphore_checks=True,
        ),
        name="attn_mod_decode",
    )(A_x, A_k_cache, A_v_cache, A_wq, A_wo, B_w_r, B_w_gate, B_w_up, B_w_down)
```

```python
import jax
import jax.numpy as jnp
from jax import lax
import jax.experimental.pallas as pl
import jax.experimental.pallas.tpu as pltpu

_HQ, _DH = 32, 128
_BF16, _F32 = jnp.bfloat16, jnp.float32
_WINDOW = 224
_STREAMS = 8
_O_FAR = 3
_INIT_P1 = 32


def _dot(a, b):
    return lax.dot_general(a, b, (((1,), (0,)), ((), ())), preferred_element_type=_F32)


def _dot_nt(a, b):
    return lax.dot_general(a, b, (((1,), (1,)), ((), ())), preferred_element_type=_F32)


def _rows(r0, nr, c0=None, nc=None):
    cols = slice(None) if c0 is None else pl.ds(c0, nc)
    return (pl.ds(r0, nr), cols)


class _CopyStream:
    def __init__(self, src, dst, sems, window):
        self.src, self.dst, self.sems, self.window = src, dst, sems, window
        self.copies = []
        self.groups = {}
        self.sem_of = {}
        self.started = 0
        self.done = 0
        self.waited = set()

    def add(self, name, src_idx, dst_idx, group):
        if group not in self.groups:
            self.groups[group] = []
            self.sem_of[group] = len(self.sem_of)
        self.groups[group].append(len(self.copies))
        self.copies.append((name, src_idx, dst_idx, group))

    def add_round_robin(self, streams, group_of):
        for r in range(max(len(s) for s in streams)):
            for j, s in enumerate(streams):
                if r < len(s):
                    self.add(*s[r], group_of(r, j))

    def _copy(self, i):
        name, src_idx, dst_idx, group = self.copies[i]
        return pltpu.make_async_copy(
            self.src[name].at[src_idx], self.dst[name].at[dst_idx], self.sems.at[self.sem_of[group]])

    def start_next(self):
        i = self.started
        self._copy(i).start(priority=1 if i < _INIT_P1 else i % 2)
        self.started += 1

    def fill(self):
        while self.started < len(self.copies) and self.started - self.done < self.window:
            self.start_next()

    def wait(self, group):
        if group in self.waited:
            return
        ids = self.groups[group]
        while self.started <= ids[-1]:
            self.start_next()
        for i in ids:
            self._copy(i).wait()
        self.waited.add(group)
        self.done += len(ids)
        self.fill()


def _plan(d, f, hkv, sk, w):
    ns = _STREAMS
    hq_dh = _HQ * _DH

    def same(name, idx):
        return (name, idx, idx)

    per = d // ns
    q_phase = [[same("wq", _rows(per * j + 8 * t, 8, (hq_dh // 2) * c, hq_dh // 2))
                for t in range(per // 8) for c in range(2)] for j in range(ns)]
    kv_phases = []
    for g in range(0, hkv, ns // 2):
        kv_phases.append([
            [(name, (0, h, pl.ds(sk - w + 128 * r, 128), slice(None)), (h, pl.ds(128 * r, 128), slice(None)))
             for r in range(w // 128)]
            for h in range(g, g + ns // 2) for name in ("k", "v")])
    ffn = [same(name, _rows(8 * t, 8)) for name in ("wg", "wu") for t in range(d // 8)]
    ffn += [same("wd", _rows(32 * r, 32)) for r in range(f // 32)]
    per = len(ffn) // ns
    assert per * ns == len(ffn)
    ffn_phase = [ffn[per * j:per * (j + 1)] for j in range(ns)]
    o_phase = [[same("wo", _rows(_DH * _O_FAR * j + 32 * r, 32)) for r in range(4 * _O_FAR)]
               for j in range(ns)]
    return q_phase, kv_phases, ffn_phase, o_phase


def _kernel(x_hbm, k_hbm, v_hbm, wq_hbm, wo_hbm, wr_hbm, wg_hbm, wu_hbm, wd_hbm, o_ref,
            x_buf, wr_buf, wq_buf, k_buf, v_buf, wo_buf, wg_buf, wu_buf, wd_buf, sems, small_sems):
    d = x_hbm.shape[-1]
    f = wg_hbm.shape[-1]
    hkv, sk = k_hbm.shape[1], k_hbm.shape[2]
    w = k_buf.shape[1]
    rep = _HQ // hkv
    ns = _STREAMS

    stream = _CopyStream(
        dict(k=k_hbm, v=v_hbm, wq=wq_hbm, wo=wo_hbm, wg=wg_hbm, wu=wu_hbm, wd=wd_hbm),
        dict(k=k_buf, v=v_buf, wq=wq_buf, wo=wo_buf, wg=wg_buf, wu=wu_buf, wd=wd_buf),
        sems, _WINDOW)
    q_phase, kv_phases, ffn_phase, o_phase = _plan(d, f, hkv, sk, w)
    rounds = []

    def by_round(tag):
        def group_of(r, _):
            if (tag, r) not in rounds:
                rounds.append((tag, r))
            return (tag, r)
        return group_of

    stream.add_round_robin(q_phase, by_round("q"))
    for g, phase in enumerate(kv_phases):
        stream.add_round_robin(phase, by_round(("kv", g)))
    stream.add_round_robin(ffn_phase, by_round("ffn"))
    assert len(stream.copies) % 2 == 0
    stream.add_round_robin(o_phase, lambda r, j: ("o", r // 4, j % 2))
    tail0 = ns * _O_FAR
    n_pairs = (_HQ - tail0) // 2
    vpu_head = _HQ - 1
    for pr in range(n_pairs):
        for c in range(4):
            for par in range(2):
                h = tail0 + 2 * pr + par
                idx = _rows(_DH * h + 32 * c, 32)
                stream.add("wo", idx, idx, ("v", c) if h == vpu_head else ("t", pr, par))

    def far(u, par):
        return [(("o", u, par), [_O_FAR * j + u for j in range(par, ns, 2)])]

    def tail(pr, par):
        return [(("t", pr, par), [tail0 + 2 * pr + par])]

    units = []
    for u in range(_O_FAR - 1):
        units += [far(u, 0), far(u, 1)]
    units += [far(_O_FAR - 1, 0), sum((tail(pr, 0) for pr in range(n_pairs)), []), far(_O_FAR - 1, 1)]
    units += [tail(pr, 1) for pr in range(n_pairs - 1)]
    units = [([g for g, _ in u], [h for _, hs in u for h in hs]) for u in units]

    def need(tag):
        last = [g for g in rounds if g[0] == tag][-1]
        for g in rounds:
            stream.wait(g)
            if g == last:
                break

    x_copy = pltpu.make_async_copy(x_hbm, x_buf, small_sems.at[0])
    wr_copy = pltpu.make_async_copy(wr_hbm, wr_buf, small_sems.at[1])
    for _ in range(ns):
        stream.start_next()
    x_copy.start()
    wr_copy.start()
    stream.fill()
    x_copy.wait()
    wr_copy.wait()

    x = x_buf[0].astype(_F32)
    xc = x - jnp.mean(x, axis=-1, keepdims=True)
    var = jnp.mean(xc * xc, axis=-1, keepdims=True)
    xn = (xc / jnp.sqrt(var + 1e-5)).astype(_BF16).astype(_F32)
    w_r = wr_buf[...].astype(_F32).reshape(1, d)
    gate = jax.nn.sigmoid(jnp.sum(xn * w_r, axis=-1, keepdims=True))
    xn8 = jnp.broadcast_to(xn, (8, d)).astype(_BF16)

    need("q")
    q = _dot(xn8, wq_buf[...])
    head_row = lax.broadcasted_iota(jnp.int32, (8, _DH), 0) % rep
    scale = _DH ** -0.5
    heads_out = []
    for g in range(len(kv_phases)):
        need(("kv", g))
        for h in range(g * (ns // 2), (g + 1) * (ns // 2)):
            q_g = q[:, rep * h * _DH:(rep * h + 1) * _DH]
            for r in range(1, rep):
                q_g = jnp.where(head_row == r, q[:, (rep * h + r) * _DH:(rep * h + r + 1) * _DH], q_g)
            s = _dot_nt(q_g.astype(_BF16), k_buf[h]) * scale
            p = jnp.exp(s - jnp.max(s, axis=-1, keepdims=True))
            denom = jnp.sum(p, axis=-1, keepdims=True)
            o = _dot(p.astype(_BF16), v_buf[h]) / denom
            heads_out.append(o.astype(_BF16).astype(_F32))

    need("ffn")
    g_act = jax.nn.silu(_dot(xn8, wg_buf[...]))
    act = (g_act * _dot(xn8, wu_buf[...])).astype(_BF16)
    y = _dot(act, wd_buf[...])

    def head(h):
        return jnp.broadcast_to(heads_out[h // rep][h % rep:h % rep + 1, :], (8, _DH))

    lhs = [jnp.concatenate([head(h) for h in hs], axis=1).astype(_BF16) for _, hs in units]
    o_col = jnp.broadcast_to(heads_out[vpu_head // rep][vpu_head % rep:vpu_head % rep + 1, :], (_DH, _DH)).T
    acc = jnp.broadcast_to(x + xn, (8, d)) + y * gate
    for (groups, hs), a in zip(units, lhs):
        for g in groups:
            stream.wait(g)
        acc = acc + _dot(a, jnp.concatenate([wo_buf[pl.ds(_DH * h, _DH), :] for h in hs], axis=0))
    acc8 = None
    for c in range(4):
        stream.wait(("v", c))
        wv = wo_buf[pl.ds(_DH * vpu_head + 32 * c, 32), :].astype(_F32)
        prod = wv * jnp.concatenate([o_col[32 * c:32 * (c + 1), :]] * (d // _DH), axis=1)
        part = (prod[0:8] + prod[8:16]) + (prod[16:24] + prod[24:32])
        acc8 = part if acc8 is None else acc8 + part
        if c == 2:
            row = lax.broadcasted_iota(jnp.int32, (8, d), 0)
            acc8 = acc8 + jnp.where(row == 0, acc, 0.0)
    assert stream.done == len(stream.copies)
    o_ref[0] = jnp.sum(acc8, axis=0, keepdims=True).astype(o_ref.dtype)


@jax.jit
def pallas_parallel_sum__sliding_block_cached__moe_arch_mod__decode_kernel(
    A_x: jax.Array,
    A_k_cache: jax.Array,
    A_v_cache: jax.Array,
    A_wq: jax.Array,
    A_wo: jax.Array,
    B_x: jax.Array,
    B_w_r: jax.Array,
    B_w_gate: jax.Array,
    B_w_up: jax.Array,
    B_w_down: jax.Array,
):
    del B_x
    b, sq, d = A_x.shape
    _, hkv, sk, dh = A_k_cache.shape
    f = B_w_gate.shape[-1]
    w = min(4096, max(256, sk // 4))
    assert (b, sq, dh, hkv) == (1, 1, _DH, _STREAMS) and A_wq.shape == (d, _HQ * _DH)
    hbm = pl.BlockSpec(memory_space=pl.ANY)
    return pl.pallas_call(
        _kernel,
        out_shape=jax.ShapeDtypeStruct((b, sq, d), A_x.dtype),
        in_specs=[hbm] * 9,
        out_specs=pl.BlockSpec(memory_space=pltpu.VMEM),
        scratch_shapes=[
            pltpu.VMEM((b, sq, d), _BF16),
            pltpu.VMEM((d,), _BF16),
            pltpu.VMEM((d, _HQ * _DH), _BF16),
            pltpu.VMEM((hkv, w, dh), _BF16),
            pltpu.VMEM((hkv, w, dh), _BF16),
            pltpu.VMEM((_HQ * _DH, d), _BF16),
            pltpu.VMEM((d, f), _BF16),
            pltpu.VMEM((d, f), _BF16),
            pltpu.VMEM((f, d), _BF16),
            pltpu.SemaphoreType.DMA((144,)),
            pltpu.SemaphoreType.DMA((2,)),
        ],
        compiler_params=pltpu.CompilerParams(
            vmem_limit_bytes=48 * 1024 * 1024,
            disable_semaphore_checks=True,
        ),
        name="attn_mod_decode",
    )(A_x, A_k_cache, A_v_cache, A_wq, A_wo, B_w_r, B_w_gate, B_w_up, B_w_down)
```
